```python
import jax
import jax.numpy as jnp

def _softmax(x, axis=-1):
    return jax.nn.softmax(x, axis=axis)

def _gelu(x):
    return jax.nn.gelu(x, approximate=True)

def _silu(x):
    return jax.nn.silu(x)

def _sigmoid(x):
    return jax.nn.sigmoid(x)

def _layernorm(x, axis=-1, eps=1e-05):
    m = jnp.mean(x, axis=axis, keepdims=True)
    v = jnp.var(x, axis=axis, keepdims=True)
    return (x - m) / jnp.sqrt(v + eps)

def _scatter_add(tgt, idx, src, axis=0):
    return tgt.at[idx].add(src)

def _segment_sum(src, seg, n):
    return jax.ops.segment_sum(src, seg, n)

class _Rng:

    def __init__(self, key):
        self._k = key

    def _next(self):
        self._k, sub = jax.random.split(self._k)
        return sub

    def normal(self, shape):
        return jax.random.normal(self._next(), shape, dtype=jnp.bfloat16)

    def randint(self, lo, hi, shape):
        return jax.random.randint(self._next(), shape, lo, hi, dtype=jnp.int32)

    def uniform(self, shape, lo=0.0, hi=1.0):
        return jax.random.uniform(self._next(), shape, jnp.bfloat16, lo, hi)

    def permutation(self, n):
        return jax.random.permutation(self._next(), n)
kernel_name = 'standalone__dilated_atrous__vision'

def setup_inputs():
    _rng = _Rng(jax.random.key(int.from_bytes(__import__("os").urandom(4), "little")))
    _w = lambda a: (lambda t: t.astype(jnp.bfloat16) if jnp.issubdtype(t.dtype, jnp.floating) else t)(jnp.asarray(a))
    H = W = 384
    C = 384
    k = 1
    return {'x': _w((lambda *s: _rng.normal(s) * 0.05)(1, H, W, C)), 'w': _w((lambda *s: _rng.normal(s) * 0.05)(k, k, C, C) * (1.0 / (k * C ** 0.5)))}

def reference(x, w):
    B, H, W, C = x.shape
    k = 1
    rate = 2
    pad = (k - 1) * rate // 2
    xp = jnp.pad(x, ((0, 0), (pad, pad), (pad, pad), (0, 0)))
    out = jnp.zeros_like(x)
    for i in range(k):
        for j in range(k):
            tap = xp[:, i * rate:i * rate + H, j * rate:j * rate + W, :].copy()
            out = out + jnp.einsum('bhwc,co->bhwo', tap, w[i, j])
    return out
```

```python
import functools

import jax
import jax.numpy as jnp
from jax import lax
import jax.experimental.pallas as pl
import jax.experimental.pallas.tpu as pltpu

_SLABS = 36
_PIECE = 32
_ROUNDS = 12
_READ_SLABS = (2, 4, 2, 4)
_CHUNK_SLABS = 6
_AHEAD = 4
_SEMS = 8
_TAIL = 4
_FIRST_WRITES = 4


def _split(i, n):
    assert n & (n - 1) == 0
    return i >> (n.bit_length() - 1), i & (n - 1)


@jax.jit
def pallas_standalone__dilated_atrous__vision_kernel(
    x: jax.Array,
    w: jax.Array,
):
    B, H, W, C = x.shape
    assert w.shape == (1, 1, C, C) and C % 128 == 0
    M = B * H * W
    blocks = C // 128
    flat = M * blocks // _SLABS
    span = _ROUNDS * _PIECE
    spans = flat // span
    read_slabs = sum(_READ_SLABS)
    n_batches = _SLABS // read_slabs * spans
    n_chunks = _SLABS // _CHUNK_SLABS * spans
    n_early = n_batches - _AHEAD
    assert spans * span * _SLABS == M * blocks and span % (16 * blocks) == 0
    assert _SLABS % read_slabs == 0 and read_slabs % _CHUNK_SLABS == 0
    assert _AHEAD < _SEMS and _FIRST_WRITES < n_early

    def kernel_function(x_hbm, w_hbm, o_hbm, buf, wbuf, sems, aux_sem, out_sem):
        def rounds(i, lo, hi):
            start = pl.multiple_of(i * span, span)
            return pl.ds(start + lo * _PIECE, (hi - lo) * _PIECE)

        def read(slabs, rows, sem):
            return pltpu.make_async_copy(
                x_hbm.at[slabs, rows], buf.at[slabs, rows], sem)

        def batch_sem(b, in_tail):
            b = b + jnp.where(b == n_batches - 1, 1, 0) if in_tail else b
            return sems.at[b & (_SEMS - 1)]

        def start_reads(b, lo, hi):
            group, i = _split(b, spans)
            for r in range(lo, hi):
                slab = group * read_slabs
                for k, n in enumerate(_READ_SLABS):
                    copy = read(pl.ds(slab, n), rounds(i, r, r + 1),
                                batch_sem(b, r >= _ROUNDS - _TAIL))
                    copy.start(priority=k % 2)
                    slab = slab + n

        def wait_reads(b, lo=0, hi=_ROUNDS):
            group, i = _split(b, spans)
            read(pl.ds(group * read_slabs, read_slabs), rounds(i, lo, hi),
                 batch_sem(b, lo > 0)).wait()

        def start_writes(c):
            group, i = _split(c, spans)
            slabs = pl.ds(group * _CHUNK_SLABS, _CHUNK_SLABS)
            for r in range(_ROUNDS):
                rows = rounds(i, r, r + 1)
                pltpu.make_async_copy(
                    buf.at[slabs, rows], o_hbm.at[slabs, rows], out_sem).start()

        def multiply(c, midway=None):
            group, i = _split(c, spans)
            rows = rounds(i, 0, _ROUNDS)
            n = _CHUNK_SLABS * span // (8 * blocks)
            v = buf[pl.ds(group * _CHUNK_SLABS, _CHUNK_SLABS), rows]
            v = v.astype(jnp.float32).reshape(n, 8 * blocks, 128)
            v = jnp.concatenate(
                [v[:, 8 * t:8 * t + 8].reshape(8 * n, 128) for t in range(blocks)],
                axis=1).astype(buf.dtype)
            v = jnp.dot(v, wbuf[...], preferred_element_type=jnp.float32)
            v = v.reshape(n, 8, C)
            v = jnp.concatenate(
                [v[:, :, 128 * t:128 * t + 128] for t in range(blocks)], axis=1)
            v = v.reshape(_CHUNK_SLABS, span, 128).astype(buf.dtype)
            half = _CHUNK_SLABS // 2
            buf[pl.ds(group * _CHUNK_SLABS, half), rows] = v[:half]
            if midway is not None:
                midway()
            buf[pl.ds(group * _CHUNK_SLABS + half, half), rows] = v[half:]

        w_copy = pltpu.make_async_copy(w_hbm, wbuf, aux_sem)
        w_copy.start()
        lax.fori_loop(0, _AHEAD, lambda b, _: start_reads(b, 0, _ROUNDS), None)
        w_copy.wait()

        def read_step(c, _):
            wait_reads(c)
            start_reads(c + _AHEAD, 0, _ROUNDS // 2)
            multiply(c, functools.partial(
                start_reads, c + _AHEAD, _ROUNDS // 2, _ROUNDS))

        lax.fori_loop(0, n_early, read_step, None)

        for b in range(n_early, n_batches - 1):
            wait_reads(b)
        wait_reads(n_batches - 1, 0, _ROUNDS - _TAIL)
        lax.fori_loop(0, _FIRST_WRITES, lambda c, _: start_writes(c), None)
        wait_reads(n_batches - 1, _ROUNDS - _TAIL, _ROUNDS)

        def write_step(c, queued):
            extra = (queued + 1 < c) & ((c & 7) != 0)

            @pl.when(extra)
            def _():
                start_writes(queued)

            queued = queued + extra.astype(jnp.int32)
            start_writes(queued)
            multiply(c)
            return queued + 1

        queued = lax.fori_loop(
            n_early, n_chunks, write_step, jnp.int32(_FIRST_WRITES))
        lax.fori_loop(queued, n_chunks, lambda c, _: start_writes(c), None)
        pltpu.make_async_copy(buf, o_hbm, out_sem).wait()

    tiles = x.reshape(M // 8, 8, blocks, 128).transpose(0, 2, 1, 3)
    out = pl.pallas_call(
        kernel_function,
        in_specs=[
            pl.BlockSpec(memory_space=pl.ANY),
            pl.BlockSpec(memory_space=pl.ANY),
        ],
        out_specs=pl.BlockSpec(memory_space=pl.ANY),
        out_shape=jax.ShapeDtypeStruct((_SLABS, flat, 128), x.dtype),
        scratch_shapes=[
            pltpu.VMEM((_SLABS, flat, 128), x.dtype),
            pltpu.VMEM((C, C), w.dtype),
            pltpu.SemaphoreType.DMA((_SEMS,)),
            pltpu.SemaphoreType.DMA(()),
            pltpu.SemaphoreType.DMA(()),
        ],
        compiler_params=pltpu.CompilerParams(
            vmem_limit_bytes=120 * 2**20,
            disable_bounds_checks=True,
            disable_semaphore_checks=True,
        ),
    )(tiles.reshape(_SLABS, flat, 128), w.reshape(C, C))
    out = out.reshape(M // 8, blocks, 8, 128).transpose(0, 2, 1, 3)
    return out.reshape(B, H, W, C)
```

```python
import functools

import jax
import jax.numpy as jnp
from jax import lax
import jax.experimental.pallas as pl
import jax.experimental.pallas.tpu as pltpu

_SLAB = 4096
_ROUND = 64
_WRITE_SLABS = 6
_READ_SLABS = 12
_READS = tuple(
    (first + s, n, row, _ROUND // 2, queue)
    for first in (0, 6)
    for row in (0, _ROUND // 2)
    for s, n, queue in ((0, 1, 0), (1, 5, 1))
)
_UNIT = 1024
_STEP_READS = (3, 2, 2)
_STEP_WRITES = 13
_LAG = 12
_TAIL = 3


def _split(i, n):
    assert n & (n - 1) == 0
    return i >> (n.bit_length() - 1), i & (n - 1)


@jax.jit
def pallas_standalone__dilated_atrous__vision_kernel(
    x: jax.Array,
    w: jax.Array,
):
    B, H, W, C = x.shape
    blocks = len(_STEP_READS)
    assert w.shape == (1, 1, C, C) and C == 128 * blocks
    M = B * H * W
    n_slabs = M * blocks // _SLAB
    n_steps = M // _UNIT
    rounds = _SLAB // _ROUND
    n_groups = n_slabs // _READ_SLABS
    n_reads = n_groups * rounds
    n_writes = n_slabs // _WRITE_SLABS * rounds
    group_steps = n_steps // n_groups
    assert n_groups * _READ_SLABS * _SLAB == M * blocks
    assert group_steps * n_groups == n_steps and _READ_SLABS % _WRITE_SLABS == 0

    step_reads = sum(_STEP_READS)
    n_early = (n_reads - _TAIL - rounds - _LAG) // step_reads
    first_reads = n_reads - _TAIL - n_early * step_reads
    first_writes = rounds
    assert step_reads * group_steps >= rounds
    for i in range(n_early, n_steps):
        done = i * blocks * _UNIT // (_WRITE_SLABS * _SLAB) * rounds
        assert first_writes + (i - n_early + 1) * _STEP_WRITES <= done

    def kernel_function(x_hbm, w_hbm, o_hbm, buf, wbuf, out_sem):
        def write(k, _=None):
            group, j = _split(k, rounds)
            slabs = pl.ds(group * _WRITE_SLABS, _WRITE_SLABS)
            rows = pl.ds(pl.multiple_of(j * _ROUND, _ROUND), _ROUND)
            pltpu.make_async_copy(
                buf.at[slabs, rows], o_hbm.at[slabs, rows], out_sem).start()

        def multiply(i, between=()):
            units = []
            for u in range(blocks):
                slab, q = _split(i * blocks + u, _SLAB // _UNIT)
                units.append((slab, pl.ds(pl.multiple_of(q * _UNIT, _UNIT), _UNIT)))
            n = _UNIT // 8
            v = jnp.concatenate([buf[unit] for unit in units], axis=0)
            v = v.astype(jnp.float32).reshape(n, 8 * blocks, 128)
            v = jnp.concatenate(
                [v[:, 8 * t:8 * t + 8].reshape(_UNIT, 128) for t in range(blocks)],
                axis=1).astype(buf.dtype)
            v = jnp.dot(v, wbuf[...], preferred_element_type=jnp.float32)
            v = v.reshape(n, 8, C)
            v = jnp.concatenate(
                [v[:, :, 128 * t:128 * t + 128] for t in range(blocks)], axis=1)
            v = v.reshape(blocks * _UNIT, 128).astype(buf.dtype)
            for u, unit in enumerate(units):
                buf[unit] = v[u * _UNIT:(u + 1) * _UNIT]
                if u < len(between):
                    between[u]()

        def read_burst(group_sems, aux_sem):
            def copy(slabs, rows, sem):
                return pltpu.make_async_copy(
                    x_hbm.at[slabs, rows], buf.at[slabs, rows], sem)

            def read(k, sem=None):
                group, j = _split(k, rounds)
                start = pl.multiple_of(j * _ROUND, _ROUND)
                for s, n, row, rows, queue in _READS:
                    copy(pl.ds(group * _READ_SLABS + s, n), pl.ds(start + row, rows),
                         group_sems.at[group] if sem is None else sem
                         ).start(priority=queue)

            def wait(group, lo, hi, sem):
                copy(pl.ds(group * _READ_SLABS, _READ_SLABS),
                     pl.ds(lo * _ROUND, (hi - lo) * _ROUND), sem).wait()

            w_copy = pltpu.make_async_copy(w_hbm, wbuf, aux_sem)
            w_copy.start()
            lax.fori_loop(0, first_reads, lambda k, _: read(k), None)
            w_copy.wait()

            def early_step(i, _):
                group, j = _split(i, group_steps)

                @pl.when(j == 0)
                def _():
                    wait(group, 0, rounds, group_sems.at[group])

                def reads(part):
                    lo = first_reads + i * step_reads + sum(_STEP_READS[:part])
                    for k in range(_STEP_READS[part]):
                        read(lo + k)

                reads(0)
                multiply(i, [functools.partial(reads, p) for p in range(1, blocks)])

            lax.fori_loop(0, n_early, early_step, None)

            for k in range(n_reads - _TAIL, n_reads):
                read(k, aux_sem)
            last = n_groups - 1
            for group in range(pl.cdiv(n_early, group_steps), last):
                wait(group, 0, rounds, group_sems.at[group])
            wait(last, 0, rounds - _TAIL, group_sems.at[last])
            lax.fori_loop(0, first_writes, write, None)
            wait(last, rounds - _TAIL, rounds, aux_sem)

        pl.run_scoped(
            read_burst,
            pltpu.SemaphoreType.DMA((n_groups,)),
            pltpu.SemaphoreType.DMA(()),
        )

        def late_step(i, _):
            for k in range(_STEP_WRITES):
                write(first_writes + (i - n_early) * _STEP_WRITES + k)
            multiply(i)

        lax.fori_loop(n_early, n_steps, late_step, None)
        queued = first_writes + (n_steps - n_early) * _STEP_WRITES
        lax.fori_loop(queued, n_writes, write, None)
        pltpu.make_async_copy(buf, o_hbm, out_sem).wait()

    tiles = x.reshape(M // 8, 8, blocks, 128).transpose(0, 2, 1, 3)
    out = pl.pallas_call(
        kernel_function,
        in_specs=[
            pl.BlockSpec(memory_space=pl.ANY),
            pl.BlockSpec(memory_space=pl.ANY),
        ],
        out_specs=pl.BlockSpec(memory_space=pl.ANY),
        out_shape=jax.ShapeDtypeStruct((n_slabs, _SLAB, 128), x.dtype),
        scratch_shapes=[
            pltpu.VMEM((n_slabs, _SLAB, 128), x.dtype),
            pltpu.VMEM((C, C), w.dtype),
            pltpu.SemaphoreType.DMA(()),
        ],
        compiler_params=pltpu.CompilerParams(vmem_limit_bytes=120 * 2**20),
    )(tiles.reshape(n_slabs, _SLAB, 128), w.reshape(C, C))
    out = out.reshape(M // 8, blocks, 8, 128).transpose(0, 2, 1, 3)
    return out.reshape(B, H, W, C)
```

```python
import functools

import jax
import jax.numpy as jnp
from jax import lax
import jax.experimental.pallas as pl
import jax.experimental.pallas.tpu as pltpu

_SLAB = 4096
_ROUND = 64
_WRITE_SLABS = 6
_READ_SLABS = 12
_HOP = 6
_UNIT = 1024
_STEP_READS = (3, 2, 2)
_STEP_WRITES = 13
_LAG = 12
_HEAD = 4
_TAIL = 3


def _split(i, n):
    assert n & (n - 1) == 0
    return i >> (n.bit_length() - 1), i & (n - 1)


@jax.jit
def pallas_standalone__dilated_atrous__vision_kernel(
    x: jax.Array,
    w: jax.Array,
):
    B, H, W, C = x.shape
    blocks = len(_STEP_READS)
    assert w.shape == (1, 1, C, C) and C == 128 * blocks
    M = B * H * W
    n_slabs = M * blocks // _SLAB
    n_steps = M // _UNIT
    rounds = _SLAB // _ROUND
    n_groups = n_slabs // _READ_SLABS
    n_reads = n_groups * rounds
    n_writes = n_slabs // _WRITE_SLABS * rounds
    group_steps = n_steps // n_groups
    assert n_groups * _READ_SLABS * _SLAB == M * blocks
    assert group_steps * n_groups == n_steps and n_slabs % _WRITE_SLABS == 0

    step_reads = sum(_STEP_READS)
    n_early = (n_reads - _TAIL - rounds - _LAG) // step_reads
    first_reads = n_reads - _TAIL - n_early * step_reads
    first_writes = rounds
    assert step_reads * group_steps >= rounds
    assert pl.cdiv(n_early, group_steps) < n_groups and _READ_SLABS % _HOP == 0
    for i in range(n_early, n_steps):
        done = i * blocks * _UNIT // (_WRITE_SLABS * _SLAB) * rounds
        assert first_writes + (i - n_early + 1) * _STEP_WRITES <= done

    half = _ROUND // 2
    visits = [(s, row) for s in range(0, _READ_SLABS, _HOP) for row in (0, half)]
    w_reads = _HEAD + C // (8 * len(visits))
    assert C % (8 * len(visits)) == 0 and w_reads <= first_reads

    def body(x_hbm, w_hbm, o_hbm, buf, wbuf, group_sems, aux_sem, out_sem):
        def copy_in(slabs, rows, sem):
            return pltpu.make_async_copy(
                x_hbm.at[slabs, rows], buf.at[slabs, rows], sem)

        def read(k, sem=None, short_copy=None):
            group, j = _split(k, rounds)
            sem = group_sems.at[group] if sem is None else sem
            for v, (s, row) in enumerate(visits):
                slab = group * _READ_SLABS + s
                rows = pl.ds(pl.multiple_of(j * _ROUND + row, half), half)
                if short_copy is None:
                    copy_in(pl.ds(slab, 1), rows, sem).start(priority=0)
                    copy_in(pl.ds(slab + 1, _HOP - 1), rows, sem).start(priority=1)
                else:
                    short_copy(v)
                    copy_in(pl.ds(slab, _HOP), rows, sem).start(priority=1)

        def read_with_w(k, _):
            def short_copy(v):
                tile_row = (k - _HEAD) * len(visits) + v
                rows = pl.ds(pl.multiple_of(8 * tile_row, 8), 8)
                pltpu.make_async_copy(
                    w_hbm.at[rows], wbuf.at[rows], aux_sem).start(priority=0)

            read(k, short_copy=short_copy)

        def wait_reads(group, lo, hi, sem):
            copy_in(pl.ds(group * _READ_SLABS, _READ_SLABS),
                    pl.ds(lo * _ROUND, (hi - lo) * _ROUND), sem).wait()

        def write(k, _=None):
            group, j = _split(k, rounds)
            slabs = pl.ds(group * _WRITE_SLABS, _WRITE_SLABS)
            rows = pl.ds(pl.multiple_of(j * _ROUND, _ROUND), _ROUND)
            pltpu.make_async_copy(
                buf.at[slabs, rows], o_hbm.at[slabs, rows], out_sem).start()

        def multiply(i, between=()):
            units = []
            for u in range(blocks):
                slab, q = _split(i * blocks + u, _SLAB // _UNIT)
                units.append((slab, pl.ds(pl.multiple_of(q * _UNIT, _UNIT), _UNIT)))
            n = _UNIT // 8
            v = jnp.concatenate([buf[unit] for unit in units], axis=0)
            v = v.astype(jnp.float32).reshape(n, 8 * blocks, 128)
            v = jnp.concatenate(
                [v[:, 8 * t:8 * t + 8].reshape(_UNIT, 128) for t in range(blocks)],
                axis=1).astype(buf.dtype)
            v = jnp.dot(v, wbuf[...], preferred_element_type=jnp.float32)
            v = v.reshape(n, 8, C)
            v = jnp.concatenate(
                [v[:, :, 128 * t:128 * t + 128] for t in range(blocks)], axis=1)
            v = v.reshape(blocks * _UNIT, 128).astype(buf.dtype)
            for u, unit in enumerate(units):
                buf[unit] = v[u * _UNIT:(u + 1) * _UNIT]
                if u < len(between):
                    between[u]()

        def early_step(i, _):
            group, j = _split(i, group_steps)

            @pl.when(j == 0)
            def _():
                wait_reads(group, 0, rounds, group_sems.at[group])

            def reads(part):
                lo = first_reads + i * step_reads + sum(_STEP_READS[:part])
                for k in range(_STEP_READS[part]):
                    read(lo + k)

            reads(0)
            multiply(i, [functools.partial(reads, p) for p in range(1, blocks)])

        def late_step(i, _):
            for k in range(_STEP_WRITES):
                write(first_writes + (i - n_early) * _STEP_WRITES + k)
            multiply(i)

        lax.fori_loop(0, _HEAD, lambda k, _: read(k, short_copy=lambda v: None), None)
        lax.fori_loop(_HEAD, w_reads, read_with_w, None)
        lax.fori_loop(w_reads, first_reads, lambda k, _: read(k), None)
        pltpu.make_async_copy(w_hbm, wbuf, aux_sem).wait()
        lax.fori_loop(0, n_early, early_step, None)

        lax.fori_loop(n_reads - _TAIL, n_reads, lambda k, _: read(k, aux_sem), None)
        last = n_groups - 1
        for group in range(pl.cdiv(n_early, group_steps), last):
            wait_reads(group, 0, rounds, group_sems.at[group])
        wait_reads(last, 0, rounds - _TAIL, group_sems.at[last])
        lax.fori_loop(0, first_writes, write, None)
        wait_reads(last, rounds - _TAIL, rounds, aux_sem)

        lax.fori_loop(n_early, n_steps, late_step, None)
        queued = first_writes + (n_steps - n_early) * _STEP_WRITES
        lax.fori_loop(queued, n_writes, write, None)
        pltpu.make_async_copy(buf, o_hbm, out_sem).wait()

    def kernel_function(*refs):
        pl.run_scoped(
            functools.partial(body, *refs),
            pltpu.SemaphoreType.DMA((n_groups,)),
            pltpu.SemaphoreType.DMA(()),
            pltpu.SemaphoreType.DMA(()),
        )

    tiles = x.reshape(M // 8, 8, blocks, 128).transpose(0, 2, 1, 3)
    out = pl.pallas_call(
        kernel_function,
        in_specs=[
            pl.BlockSpec(memory_space=pl.ANY),
            pl.BlockSpec(memory_space=pl.ANY),
        ],
        out_specs=pl.BlockSpec(memory_space=pl.ANY),
        out_shape=jax.ShapeDtypeStruct((n_slabs, _SLAB, 128), x.dtype),
        scratch_shapes=[
            pltpu.VMEM((n_slabs, _SLAB, 128), x.dtype),
            pltpu.VMEM((C, C), w.dtype),
        ],
        compiler_params=pltpu.CompilerParams(vmem_limit_bytes=120 * 2**20),
    )(tiles.reshape(n_slabs, _SLAB, 128), w.reshape(C, C))
    out = out.reshape(M // 8, blocks, 8, 128).transpose(0, 2, 1, 3)
    return out.reshape(B, H, W, C)
```

```python
import functools

import jax
import jax.numpy as jnp
from jax import lax
import jax.experimental.pallas as pl
import jax.experimental.pallas.tpu as pltpu

_SLAB = 4096
_ROUND = 64
_WRITE_SLABS = 6
_READ_SLABS = 12
_HOP = 4
_BACKLOG = 9
_UNIT = 1024
_STEP_READS = (2, 3, 2)
_STEP_WRITES = 13
_SLACK = 12
_TAIL = 3


def _split(i, n):
    assert n & (n - 1) == 0
    return i >> (n.bit_length() - 1), i & (n - 1)


@jax.jit
def pallas_standalone__dilated_atrous__vision_kernel(
    x: jax.Array,
    w: jax.Array,
):
    B, H, W, C = x.shape
    blocks = len(_STEP_READS)
    assert w.shape == (1, 1, C, C) and C == 128 * blocks
    M = B * H * W
    n_slabs = M * blocks // _SLAB
    n_steps = M // _UNIT
    rounds = _SLAB // _ROUND
    n_groups = n_slabs // _READ_SLABS
    n_reads = n_groups * rounds
    n_writes = n_slabs // _WRITE_SLABS * rounds
    group_steps = n_steps // n_groups
    assert n_groups * _READ_SLABS * _SLAB == M * blocks
    assert group_steps * n_groups == n_steps and n_slabs % _WRITE_SLABS == 0
    assert _READ_SLABS % _HOP == 0 and _TAIL <= _BACKLOG

    step_reads = sum(_STEP_READS)
    tail = n_reads - _TAIL
    n_early = (tail - rounds - _BACKLOG - _SLACK) // step_reads
    first_reads = tail - n_early * step_reads
    first_writes = rounds
    assert step_reads * group_steps >= rounds
    assert pl.cdiv(n_early, group_steps) < n_groups
    for i in range(n_early, n_steps):
        done = i * blocks * _UNIT // (_WRITE_SLABS * _SLAB) * rounds
        assert first_writes + (i - n_early + 1) * _STEP_WRITES <= done

    def body(x_hbm, w_hbm, o_hbm, buf, wbuf, group_sems, aux_sem, out_sem):
        def copy_in(slabs, rows, sem):
            return pltpu.make_async_copy(
                x_hbm.at[slabs, rows], buf.at[slabs, rows], sem)

        def start_in(k, slab, slabs, queue):
            group, j = _split(k, rounds)
            in_tail = isinstance(k, int) and k >= tail
            copy_in(pl.ds(group * _READ_SLABS + slab, slabs),
                    pl.ds(pl.multiple_of(j * _ROUND, _ROUND), _ROUND),
                    aux_sem if in_tail else group_sems.at[group]
                    ).start(priority=queue)

        def read(k, _=None, short=True, long=True):
            for s in range(0, _READ_SLABS, _HOP):
                if short:
                    start_in(k - _BACKLOG, s + _HOP - 1, 1, queue=0)
                if long:
                    start_in(k, s, _HOP - 1, queue=1)

        def wait_reads(group, lo, hi, sem):
            copy_in(pl.ds(group * _READ_SLABS, _READ_SLABS),
                    pl.ds(lo * _ROUND, (hi - lo) * _ROUND), sem).wait()

        def write(k, _=None):
            group, j = _split(k, rounds)
            slabs = pl.ds(group * _WRITE_SLABS, _WRITE_SLABS)
            rows = pl.ds(pl.multiple_of(j * _ROUND, _ROUND), _ROUND)
            pltpu.make_async_copy(
                buf.at[slabs, rows], o_hbm.at[slabs, rows], out_sem).start()

        def multiply(i, between=()):
            units = []
            for u in range(blocks):
                slab, q = _split(i * blocks + u, _SLAB // _UNIT)
                units.append((slab, pl.ds(pl.multiple_of(q * _UNIT, _UNIT), _UNIT)))
            n = _UNIT // 8
            v = jnp.concatenate([buf[unit] for unit in units], axis=0)
            v = v.astype(jnp.float32).reshape(n, 8 * blocks, 128)
            v = jnp.concatenate(
                [v[:, 8 * t:8 * t + 8].reshape(_UNIT, 128) for t in range(blocks)],
                axis=1).astype(buf.dtype)
            v = jnp.dot(v, wbuf[...], preferred_element_type=jnp.float32)
            v = v.reshape(n, 8, C)
            v = jnp.concatenate(
                [v[:, :, 128 * t:128 * t + 128] for t in range(blocks)], axis=1)
            v = v.reshape(blocks * _UNIT, 128).astype(buf.dtype)
            for u, unit in enumerate(units):
                buf[unit] = v[u * _UNIT:(u + 1) * _UNIT]
                if u < len(between):
                    between[u]()

        def early_step(i, _):
            group, j = _split(i, group_steps)

            @pl.when(j == 0)
            def _():
                wait_reads(group, 0, rounds, group_sems.at[group])

            def reads(part):
                lo = first_reads + i * step_reads + sum(_STEP_READS[:part])
                for k in range(_STEP_READS[part]):
                    read(lo + k)

            reads(0)
            multiply(i, [functools.partial(reads, p) for p in range(1, blocks)])

        def late_step(i, _):
            for k in range(_STEP_WRITES):
                write(first_writes + (i - n_early) * _STEP_WRITES + k)
            multiply(i)

        w_copy = pltpu.make_async_copy(w_hbm, wbuf, aux_sem)
        w_copy.start()
        lax.fori_loop(0, _BACKLOG, functools.partial(read, short=False), None)
        lax.fori_loop(_BACKLOG, first_reads, read, None)
        w_copy.wait()
        lax.fori_loop(0, n_early, early_step, None)

        for k in range(tail, n_reads + _BACKLOG):
            read(k, long=k < n_reads)
        last = n_groups - 1
        for group in range(pl.cdiv(n_early, group_steps), last):
            wait_reads(group, 0, rounds, group_sems.at[group])
        wait_reads(last, 0, rounds - _TAIL, group_sems.at[last])
        lax.fori_loop(0, first_writes, write, None)
        wait_reads(last, rounds - _TAIL, rounds, aux_sem)

        lax.fori_loop(n_early, n_steps, late_step, None)
        queued = first_writes + (n_steps - n_early) * _STEP_WRITES
        lax.fori_loop(queued, n_writes, write, None)
        pltpu.make_async_copy(buf, o_hbm, out_sem).wait()

    def kernel_function(*refs):
        pl.run_scoped(
            functools.partial(body, *refs),
            pltpu.SemaphoreType.DMA((n_groups,)),
            pltpu.SemaphoreType.DMA(()),
            pltpu.SemaphoreType.DMA(()),
        )

    tiles = x.reshape(M // 8, 8, blocks, 128).transpose(0, 2, 1, 3)
    out = pl.pallas_call(
        kernel_function,
        in_specs=[
            pl.BlockSpec(memory_space=pl.ANY),
            pl.BlockSpec(memory_space=pl.ANY),
        ],
        out_specs=pl.BlockSpec(memory_space=pl.ANY),
        out_shape=jax.ShapeDtypeStruct((n_slabs, _SLAB, 128), x.dtype),
        scratch_shapes=[
            pltpu.VMEM((n_slabs, _SLAB, 128), x.dtype),
            pltpu.VMEM((C, C), w.dtype),
        ],
        compiler_params=pltpu.CompilerParams(vmem_limit_bytes=120 * 2**20),
    )(tiles.reshape(n_slabs, _SLAB, 128), w.reshape(C, C))
    out = out.reshape(M // 8, blocks, 8, 128).transpose(0, 2, 1, 3)
    return out.reshape(B, H, W, C)
```
